```python
import jax
import jax.numpy as jnp

def _softmax(x, axis=-1):
    return jax.nn.softmax(x, axis=axis)

def _gelu(x):
    return jax.nn.gelu(x, approximate=True)

def _silu(x):
    return jax.nn.silu(x)

def _sigmoid(x):
    return jax.nn.sigmoid(x)

def _layernorm(x, axis=-1, eps=1e-05):
    m = jnp.mean(x, axis=axis, keepdims=True)
    v = jnp.var(x, axis=axis, keepdims=True)
    return (x - m) / jnp.sqrt(v + eps)

def _scatter_add(tgt, idx, src, axis=0):
    return tgt.at[idx].add(src)

def _segment_sum(src, seg, n):
    return jax.ops.segment_sum(src, seg, n)

class _Rng:

    def __init__(self, key):
        self._k = key

    def _next(self):
        self._k, sub = jax.random.split(self._k)
        return sub

    def normal(self, shape):
        return jax.random.normal(self._next(), shape, dtype=jnp.bfloat16)

    def randint(self, lo, hi, shape):
        return jax.random.randint(self._next(), shape, lo, hi, dtype=jnp.int32)

    def uniform(self, shape, lo=0.0, hi=1.0):
        return jax.random.uniform(self._next(), shape, jnp.bfloat16, lo, hi)

    def permutation(self, n):
        return jax.random.permutation(self._next(), n)
kernel_name = 'concat_heads__compressed_kv_cla__memory_aug_recurrent_mem_tr__prompt'

def setup_inputs():
    _rng = _Rng(jax.random.key(int.from_bytes(__import__("os").urandom(4), "little")))
    _w = lambda a: (lambda t: t.astype(jnp.bfloat16) if jnp.issubdtype(t.dtype, jnp.floating) else t)(jnp.asarray(a))

    def _A_setup():
        B, H, Sq, Sk, D, M = (1, 32, 2048, 2048, 128, 576)
        Dc = 4 * D
        return {'x': _w((lambda *s: _rng.normal(s) * 0.05)(B, Sq, M)), 'c_kv': _w((lambda *s: _rng.normal(s) * 0.05)(B, Sk, Dc)), 'w_q': _w((lambda *s: _rng.normal(s) * 0.05)(M, H, D) * M ** (-0.5)), 'w_uk': _w((lambda *s: _rng.normal(s) * 0.05)(Dc, H, D) * Dc ** (-0.5)), 'w_uv': _w((lambda *s: _rng.normal(s) * 0.05)(Dc, H, D) * Dc ** (-0.5)), 'w_o': _w((lambda *s: _rng.normal(s) * 0.05)(H, D, M) * (H * D) ** (-0.5))}
    _A_in = _A_setup()

    def _B_setup():
        B, S, Dm = (1, 2048, 576)
        H, Dh = (32, 128)
        M, seg = (8, 32)
        seg = min(seg, S)
        S = S // seg * seg
        return {'x': _w((lambda *s: _rng.normal(s) * 0.05)(B, S, Dm)), 'mem0': _w((lambda *s: _rng.normal(s) * 0.05)(B, M, Dm)), 'Wq': _w((lambda *s: _rng.normal(s) * 0.05)(Dm, H, Dh) * Dm ** (-0.5)), 'Wk': _w((lambda *s: _rng.normal(s) * 0.05)(Dm, H, Dh) * Dm ** (-0.5)), 'Wv': _w((lambda *s: _rng.normal(s) * 0.05)(Dm, H, Dh) * Dm ** (-0.5)), 'Wo': _w((lambda *s: _rng.normal(s) * 0.05)(H, Dh, Dm) * (H * Dh) ** (-0.5)), 'seg_len': seg}
    _B_in = _B_setup()
    return {'A_x': _A_in['x'], 'A_c_kv': _A_in['c_kv'], 'A_w_q': _A_in['w_q'], 'A_w_uk': _A_in['w_uk'], 'A_w_uv': _A_in['w_uv'], 'A_w_o': _A_in['w_o'], 'B_x': _B_in['x'], 'B_mem0': _B_in['mem0'], 'B_Wq': _B_in['Wq'], 'B_Wk': _B_in['Wk'], 'B_Wv': _B_in['Wv'], 'B_Wo': _B_in['Wo'], 'B_seg_len': _B_in['seg_len']}

def reference(A_x, A_c_kv, A_w_q, A_w_uk, A_w_uv, A_w_o, B_x, B_mem0, B_Wq, B_Wk, B_Wv, B_Wo, B_seg_len):

    def _A_ref(x, c_kv, w_q, w_uk, w_uv, w_o):
        B, Sq, M = (x.shape[0], x.shape[1], x.shape[2])
        Sk = c_kv.shape[1]
        H, D = (w_q.shape[1], w_q.shape[2])
        q = jnp.einsum('bqm,mhd->bhqd', x, w_q)
        k = jnp.einsum('bkc,chd->bhkd', c_kv, w_uk)
        v = jnp.einsum('bkc,chd->bhkd', c_kv, w_uv)
        scores = jnp.einsum('bhqd,bhkd->bhqk', q, k) * D ** (-0.5)
        off = Sk - Sq
        qi = jnp.arange(Sq)[:, None]
        kj = jnp.arange(Sk)[None, :]
        cmask = kj <= qi + off
        scores = jnp.where(cmask[None, None], scores, -1000000000.0)
        p = _softmax(scores, axis=-1)
        ctx = jnp.einsum('bhqk,bhkd->bhqd', p, v)
        return jnp.einsum('bhqd,hdm->bqm', ctx, w_o)

    def _B_ref(x, mem0, Wq, Wk, Wv, Wo, seg_len):
        B, S, Dm = x.shape
        H, Dh = (Wq.shape[1], Wq.shape[2])
        M = mem0.shape[1]
        scale = Dh ** (-0.5)
        n_seg = S // seg_len
        L = M + seg_len
        idx = jnp.arange(L)
        mask = (idx[:, None] < M) | (idx[:, None] >= idx[None, :])
        mem = mem0
        outs = []
        for s in range(n_seg):
            xs = x[:, s * seg_len:(s + 1) * seg_len, :].copy()
            h = jnp.concatenate([mem, xs], axis=1)
            q = jnp.einsum('btd,dhe->bhte', h, Wq)
            k = jnp.einsum('btd,dhe->bhte', h, Wk)
            v = jnp.einsum('btd,dhe->bhte', h, Wv)
            scores = jnp.einsum('bhqe,bhke->bhqk', q, k) * scale
            scores = jnp.where(mask[None, None], scores, -1000000000.0)
            p = _softmax(scores, axis=-1)
            o = jnp.einsum('bhqk,bhke->bhqe', p, v)
            o = jnp.einsum('bhte,hed->btd', o, Wo)
            mem = o[:, :M, :].copy()
            outs.append(o[:, M:, :])
        return jnp.concatenate(outs, axis=1)
    a = _A_ref(A_x, A_c_kv, A_w_q, A_w_uk, A_w_uv, A_w_o)
    b = _B_ref(B_x, B_mem0, B_Wq, B_Wk, B_Wv, B_Wo, B_seg_len)
    return jnp.concatenate([a, b], axis=-1)
```

```python
import functools

import jax
import jax.numpy as jnp
import jax.experimental.pallas as pl
import jax.experimental.pallas.tpu as pltpu

BQ = 256
NT = (((1,), (1,)), ((), ()))


def _kernel(xa_ref, c_ref, wq_ref, wuk_ref, wuv_ref, woa_ref,
            xb_ref, mem0_ref, bq_ref, bk_ref, bv_ref, wob_ref,
            o_ref,
            wq_s, wuk_s, wuv_s, ctx_s, bw_s, xa_s, xb_s, *, seg):
    DM, S = xa_ref.shape
    H = wq_ref.shape[1]
    D = wq_ref.shape[2]
    DC = c_ref.shape[1]
    M = mem0_ref.shape[0]
    L = M + seg
    f32, bf16 = jnp.float32, jnp.bfloat16
    LOG2E = 1.4426950408889634
    scale = D ** -0.5

    for src, dst in ((wq_ref, wq_s), (wuk_ref, wuk_s), (wuv_ref, wuv_s)):
        for m in range(0, src.shape[0], 64):
            dst[:, m:m + 64, :] = jnp.swapaxes(src[m:m + 64], 0, 1)
    for t, src in enumerate((bq_ref, bk_ref, bv_ref)):
        for m in range(0, src.shape[0], 64):
            blk = jnp.swapaxes(src[m:m + 64], 0, 1)
            for h in range(H):
                bw_s[m:m + 64, (t * H + h) * D:(t * H + h + 1) * D] = blk[h]

    for i in range(0, S, 256):
        xa_s[i:i + 256, :] = xa_ref[:, i:i + 256].T
        xb_s[i:i + 256, :] = xb_ref[:, i:i + 256].T

    def head_body(h, carry):
        q = jnp.dot(xa_s[...], wq_s[h], preferred_element_type=f32)
        q = (q * (scale * LOG2E)).astype(bf16)
        k = jnp.dot(c_ref[...], wuk_s[h], preferred_element_type=f32).astype(bf16)
        v = jnp.dot(c_ref[...], wuv_s[h], preferred_element_type=f32).astype(bf16)
        row = jax.lax.broadcasted_iota(jnp.int32, (BQ, BQ), 0)
        col = jax.lax.broadcasted_iota(jnp.int32, (BQ, BQ), 1)
        for i in range(S // BQ):
            e = (i + 1) * BQ
            qi = q[i * BQ:e]
            sd = jax.lax.dot_general(qi, k[i * BQ:e], NT, preferred_element_type=f32)
            sd = jnp.where(col <= row, sd, -1e9)
            if i > 0:
                so = jax.lax.dot_general(qi, k[:i * BQ], NT, preferred_element_type=f32)
                s = jnp.concatenate([so, sd], axis=1)
            else:
                s = sd
            mx = jnp.max(s, axis=1, keepdims=True)
            p = jnp.exp2(s - mx)
            l = jnp.sum(p, axis=1, keepdims=True)
            o = jnp.dot(p.astype(bf16), v[:e], preferred_element_type=f32)
            ctx_s[h, i * BQ:e, :] = (o / l).astype(bf16)
        return carry

    jax.lax.fori_loop(0, H, head_body, 0)
    for i in range(0, S, 512):
        acc = jnp.zeros((512, DM), f32)
        for h in range(H):
            acc += jax.lax.dot_general(ctx_s[h, i:i + 512, :], woa_ref[h], NT, preferred_element_type=f32)
        o_ref[i:i + 512, :DM] = acc.astype(o_ref.dtype)

    rowi = jax.lax.broadcasted_iota(jnp.int32, (L, L), 0)
    coli = jax.lax.broadcasted_iota(jnp.int32, (L, L), 1)
    mask = (rowi < M) | (rowi >= coli)

    def step(s, mem):
        xs = xb_s[pl.ds(pl.multiple_of(s * seg, seg), seg), :]
        hh = jnp.concatenate([mem.astype(f32), xs.astype(f32)], axis=0).astype(bf16)
        qkv = jnp.dot(hh, bw_s[...], preferred_element_type=f32)
        acc = jnp.zeros((L, DM), f32)
        for h in range(H):
            q = (qkv[:, h * D:(h + 1) * D] * (scale * LOG2E)).astype(bf16)
            k = qkv[:, (H + h) * D:(H + h + 1) * D].astype(bf16)
            v = qkv[:, (2 * H + h) * D:(2 * H + h + 1) * D].astype(bf16)
            sc = jax.lax.dot_general(q, k, NT, preferred_element_type=f32)
            sc = jnp.where(mask, sc, -1e9)
            mx = jnp.max(sc, axis=1, keepdims=True)
            p = jnp.exp2(sc - mx)
            l = jnp.sum(p, axis=1, keepdims=True)
            o = jnp.dot(p.astype(bf16), v, preferred_element_type=f32) / l
            acc += jax.lax.dot_general(o.astype(bf16), wob_ref[h], NT, preferred_element_type=f32)
        o_ref[pl.ds(pl.multiple_of(s * seg, seg), seg), DM:] = acc[M:].astype(o_ref.dtype)
        return acc[:M].astype(bf16)

    jax.lax.fori_loop(0, S // seg, step, mem0_ref[...])


@functools.partial(jax.jit, static_argnames=("B_seg_len",))
def pallas_concat_heads__compressed_kv_cla__memory_aug_recurrent_mem_tr__prompt_kernel(
    A_x, A_c_kv, A_w_q, A_w_uk, A_w_uv, A_w_o,
    B_x, B_mem0, B_Wq, B_Wk, B_Wv, B_Wo, B_seg_len,
):
    Bn, S, DM = A_x.shape
    assert Bn == 1
    H, D = A_w_q.shape[1], A_w_q.shape[2]
    DC = A_c_kv.shape[2]
    M = B_mem0.shape[1]
    out = pl.pallas_call(
        functools.partial(_kernel, seg=B_seg_len),
        out_shape=jax.ShapeDtypeStruct((S, 2 * DM), jnp.bfloat16),
        scratch_shapes=[
            pltpu.VMEM((H, DM, D), jnp.bfloat16),
            pltpu.VMEM((H, DC, D), jnp.bfloat16),
            pltpu.VMEM((H, DC, D), jnp.bfloat16),
            pltpu.VMEM((H, S, D), jnp.bfloat16),
            pltpu.VMEM((DM, 3 * H * D), jnp.bfloat16),
            pltpu.VMEM((S, DM), jnp.bfloat16),
            pltpu.VMEM((S, DM), jnp.bfloat16),
        ],
        compiler_params=pltpu.CompilerParams(vmem_limit_bytes=120 * 2**20),
    )(A_x.reshape(S, DM).T, A_c_kv.reshape(S, DC), A_w_q, A_w_uk, A_w_uv, jnp.swapaxes(A_w_o, 1, 2),
      B_x.reshape(S, DM).T, B_mem0.reshape(M, DM), B_Wq, B_Wk, B_Wv, jnp.swapaxes(B_Wo, 1, 2))
    return out.reshape(1, S, 2 * DM)
```

```python
import functools

import jax
import jax.numpy as jnp
import jax.experimental.pallas as pl
import jax.experimental.pallas.tpu as pltpu

f32, bf16, u32 = jnp.float32, jnp.bfloat16, jnp.uint32
NT = (((1,), (1,)), ((), ()))
LOG2E = 1.4426950408889634
BQ = 256
G = 2
FOLD_OUT = False


def _half(x, odd):
    y = (x >> (16 * odd).astype(u32)) << 16
    return pltpu.bitcast(y, f32).astype(bf16)


def _kernel(xa_hbm, c_hbm, wq_hbm, wuk_hbm, wuv_hbm, woa_hbm,
            xb_hbm, mem0_hbm, bq_hbm, bk_hbm, bv_hbm, wob_hbm,
            o_hbm,
            xt_s, xa_s, c_s, aw_s, woa_s, acc_s, ctx_s, xb_s, mem_s, bst_s, bw_s, wob_s, out_s,
            sem_in, sem_aw, sem_bw, sem_out):
    DM, S = xa_hbm.shape
    H, D = wq_hbm.shape[1], wq_hbm.shape[2]
    DC = c_hbm.shape[1]
    KP = 640
    PAD = KP - DM
    NK = KP // 128
    M = mem0_hbm.shape[0]
    cq = (D ** -0.5) * LOG2E

    aw32 = [w.bitcast(u32) for w in (wq_hbm, wuk_hbm, wuv_hbm)]
    bw32 = [w.bitcast(u32) for w in (bq_hbm, bk_hbm, bv_hbm)]

    def aw_copy(t, h, slot):
        k = aw32[t].shape[0]
        return pltpu.make_async_copy(aw32[t].at[:, h // 2, :], aw_s.at[slot, t, pl.ds(0, k), :],
                                     sem_aw.at[slot, t])

    def bw_copy(t, p):
        return pltpu.make_async_copy(bw32[t].at[:, p, :], bst_s.at[t, p], sem_bw.at[t, p])

    cp_xa = pltpu.make_async_copy(xa_hbm, xt_s.at[0, pl.ds(0, DM), :], sem_in.at[0])
    cp_c = pltpu.make_async_copy(c_hbm, c_s, sem_in.at[1])
    cp_woa = pltpu.make_async_copy(woa_hbm, woa_s.at[:, pl.ds(0, DM), :], sem_in.at[2])
    cp_xb = pltpu.make_async_copy(xb_hbm, xt_s.at[1, pl.ds(PAD, DM), :], sem_in.at[3])
    cp_wob = pltpu.make_async_copy(wob_hbm, wob_s.at[:, pl.ds(PAD, DM), :], sem_in.at[4])
    cp_mem = pltpu.make_async_copy(mem0_hbm, mem_s, sem_in.at[5])

    cp_c.start()
    for t in (1, 2, 0):
        aw_copy(t, 0, 0).start()
    cp_xa.start()
    cp_woa.start()
    for p in range(H // 2):
        for t in range(3):
            bw_copy(t, p).start()
    cp_xb.start()
    cp_wob.start()
    cp_mem.start()

    xt_s[0, DM:, :] = jnp.zeros((PAD, S), bf16)
    xt_s[1, :PAD, :] = jnp.zeros((PAD, S), bf16)
    woa_s[:, DM:, :] = jnp.zeros((H, PAD, D), bf16)
    wob_s[:, :PAD, :] = jnp.zeros((H, PAD, D), bf16)
    for sl in range(2):
        aw_s[sl, 0, DM:, :] = jnp.zeros((PAD, D), u32)
    cp_c.wait()
    cp_xa.wait()
    for t in range(NK):
        for i in range(0, S, 256):
            xa_s[t, i:i + 256, :] = xt_s[0, t * 128:(t + 1) * 128, i:i + 256].T
    cp_woa.wait()

    row = jax.lax.broadcasted_iota(jnp.int32, (BQ, BQ), 0)
    col = jax.lax.broadcasted_iota(jnp.int32, (BQ, BQ), 1)

    def head_body(h, carry):
        slot = h % 2
        odd = h % 2
        for t in range(3):
            aw_copy(t, h, slot).wait()

        @pl.when(h + 1 < H)
        def _():
            for t in range(3):
                aw_copy(t, h + 1, 1 - slot).start()

        @pl.when(odd == 0)
        def _():
            for t in range(3):
                bw_copy(t, h // 2).wait()

        cc = c_s[...]
        k = jnp.dot(cc, _half(aw_s[slot, 1, :DC, :], odd), preferred_element_type=f32).astype(bf16)
        v = jnp.dot(cc, _half(aw_s[slot, 2, :DC, :], odd), preferred_element_type=f32).astype(bf16)
        xx = jnp.concatenate([xa_s[t] for t in range(NK)], axis=1)
        q = jnp.dot(xx, _half(aw_s[slot, 0], odd), preferred_element_type=f32)
        q = (q * cq).astype(bf16)
        for t in range(3):
            bw_s[3 * h + t, pl.ds(0, PAD), :] = jnp.zeros((PAD, D), bf16)
            bw_s[3 * h + t, pl.ds(PAD, DM), :] = _half(bst_s[t, h // 2], odd)
        for i in range(S // BQ):
            e = (i + 1) * BQ
            qi = q[i * BQ:e]
            sd = jax.lax.dot_general(qi, k[i * BQ:e], NT, preferred_element_type=f32)
            sd = jnp.where(col <= row, sd, -1e9)
            if i > 0:
                so = jax.lax.dot_general(qi, k[:i * BQ], NT, preferred_element_type=f32)
                s = jnp.concatenate([so, sd], axis=1)
            else:
                s = sd
            p = jnp.exp2(s - jnp.max(s, axis=1, keepdims=True))
            l = jnp.sum(p, axis=1, keepdims=True)
            o = jnp.dot(p.astype(bf16), v[:e], preferred_element_type=f32)
            o = (o * pl.reciprocal(l, approx=False)).astype(bf16)
            if FOLD_OUT:
                t_ = jax.lax.dot_general(o, woa_s[h], NT, preferred_element_type=f32)
                acc_s[i * BQ:e, :] = jnp.where(h == 0, t_, acc_s[i * BQ:e, :] + t_)
            else:
                ctx_s[h, i * BQ:e, :] = o
        return carry

    if FOLD_OUT:
        acc_s[...] = jnp.zeros(acc_s.shape, f32)
    jax.lax.fori_loop(0, H, head_body, 0)
    if FOLD_OUT:
        out_s[:, :KP] = acc_s[...].astype(bf16)
    else:
        def oa(i, carry):
            r = pl.ds(pl.multiple_of(i * 256, 256), 256)
            acc = None
            for h in range(H):
                t_ = jax.lax.dot_general(ctx_s[h, r, :], woa_s[h], NT, preferred_element_type=f32)
                acc = t_ if acc is None else acc + t_
            out_s[r, :KP] = acc.astype(bf16)
            return carry
        jax.lax.fori_loop(0, S // 256, oa, 0)

    cp_xb.wait()
    cp_wob.wait()
    cp_mem.wait()
    for t in range(NK):
        for i in range(0, S, 256):
            xb_s[t, i:i + 256, :] = xt_s[1, t * 128:(t + 1) * 128, i:i + 256].T

    L = 48
    r_ = jax.lax.broadcasted_iota(jnp.int32, (L, L), 0)
    c_ = jax.lax.broadcasted_iota(jnp.int32, (L, L), 1)
    maskA = ((r_ < 8) | (r_ >= c_)) & (c_ < 40)
    maskB = (((r_ >= 16) & (r_ < 24)) | ((c_ >= 16) & (c_ < 24)) | (r_ >= c_)) & (c_ >= 8)
    n = H // G

    def run(hh, mask, prevqkv, prevo):
        acc = [None]
        keep, keepo = {}, {}

        def proj(g):
            out = []
            for h in range(g * G, (g + 1) * G):
                q = (jnp.dot(hh, bw_s[3 * h], preferred_element_type=f32) * cq).astype(bf16)
                k = jnp.dot(hh, bw_s[3 * h + 1], preferred_element_type=f32).astype(bf16)
                v = jnp.dot(hh, bw_s[3 * h + 2], preferred_element_type=f32).astype(bf16)
                if prevqkv is None:
                    keep[h] = (q[32:48], k[32:48], v[32:48])
                else:
                    pq, pk, pv_ = prevqkv[h]
                    q = jnp.concatenate([pq, q], 0)
                    k = jnp.concatenate([pk, k], 0)
                    v = jnp.concatenate([pv_, v], 0)
                out.append((q, k, v))
            return out

        def qk(qkv):
            return [(jax.lax.dot_general(q, k, NT, preferred_element_type=f32), v) for q, k, v in qkv]

        def sm(sv):
            out = []
            for sc, v in sv:
                sc = jnp.where(mask, sc, -1e9)
                p = jnp.exp2(sc - jnp.max(sc, axis=1, keepdims=True))
                l = jnp.sum(p, axis=1, keepdims=True)
                out.append((p.astype(bf16), pl.reciprocal(l, approx=False), v))
            return out

        def pv(ps, g):
            out = []
            for j, (p, r, v) in enumerate(ps):
                h = g * G + j
                o = jnp.dot(p, v, preferred_element_type=f32) * r
                if prevo is None:
                    keepo[h] = o[32:40]
                    out.append(o[0:32].astype(bf16))
                else:
                    out.append(jnp.concatenate([prevo[h], o[8:48]], 0).astype(bf16))
            return out

        def wo(os, g):
            for j, o in enumerate(os):
                t_ = jax.lax.dot_general(o, wob_s[g * G + j], NT, preferred_element_type=f32)
                acc[0] = t_ if acc[0] is None else acc[0] + t_

        st = {}
        for t in range(n + 4):
            if t < n:
                st[('p', t)] = proj(t)
            if 0 <= t - 1 < n:
                st[('s', t - 1)] = qk(st.pop(('p', t - 1)))
            if 0 <= t - 2 < n:
                st[('m', t - 2)] = sm(st.pop(('s', t - 2)))
            if 0 <= t - 3 < n:
                st[('o', t - 3)] = pv(st.pop(('m', t - 3)), t - 3)
            if 0 <= t - 4 < n:
                wo(st.pop(('o', t - 4)), t - 4)
        return acc[0], keep, keepo

    def out_copy(j):
        r = pl.ds(pl.multiple_of(j * 64, 64), 64)
        return pltpu.make_async_copy(out_s.at[r, :], o_hbm.at[r, :], sem_out)

    def step(j, mem):
        r = pl.ds(pl.multiple_of(j * 64, 64), 64)
        X = jnp.concatenate([xb_s[t, r, :] for t in range(NK)], axis=1).astype(f32)
        hhA = jnp.concatenate([mem, X[0:40]], 0).astype(bf16)
        accA, keep, keepo = run(hhA, maskA, None, None)
        hhB = jnp.concatenate([accA[0:8], X[40:64]], 0).astype(bf16)
        accB, _, _ = run(hhB, maskB, keep, keepo)
        out = jnp.concatenate([accA[8:32], accB[0:16], accB[24:48]], 0)
        c0 = DM - PAD
        first = out[:, :128] + out_s[r, c0:c0 + 128].astype(f32)
        out_s[r, c0:c0 + 128] = first.astype(bf16)
        out_s[r, c0 + 128:] = out[:, 128:].astype(bf16)
        out_copy(j).start()
        return accB[16:24]

    mem0 = jnp.concatenate([jnp.zeros((M, PAD), f32), mem_s[...].astype(f32)], axis=1)
    jax.lax.fori_loop(0, S // 64, step, mem0)
    pltpu.make_async_copy(out_s, o_hbm, sem_out).wait()


@functools.partial(jax.jit, static_argnames=("B_seg_len",))
def pallas_concat_heads__compressed_kv_cla__memory_aug_recurrent_mem_tr__prompt_kernel(
    A_x, A_c_kv, A_w_q, A_w_uk, A_w_uv, A_w_o,
    B_x, B_mem0, B_Wq, B_Wk, B_Wv, B_Wo, B_seg_len,
):
    Bn, S, DM = A_x.shape
    H, D = A_w_q.shape[1], A_w_q.shape[2]
    DC = A_c_kv.shape[2]
    M = B_mem0.shape[1]
    assert (Bn, DM, D, M, B_seg_len) == (1, 576, 128, 8, 32)
    KP = 640
    any_spec = pl.BlockSpec(memory_space=pl.ANY)
    out = pl.pallas_call(
        _kernel,
        out_shape=jax.ShapeDtypeStruct((S, 2 * DM), bf16),
        in_specs=[any_spec] * 12,
        out_specs=any_spec,
        scratch_shapes=[
            pltpu.VMEM((2, KP, S), bf16),
            pltpu.VMEM((KP // 128, S, 128), bf16),
            pltpu.VMEM((S, DC), bf16),
            pltpu.VMEM((2, 3, KP, D), u32),
            pltpu.VMEM((H, KP, D), bf16),
            pltpu.VMEM((S, KP), f32) if FOLD_OUT else pltpu.VMEM((8, 128), f32),
            pltpu.VMEM((8, 16, 128), bf16) if FOLD_OUT else pltpu.VMEM((H, S, D), bf16),
            pltpu.VMEM((KP // 128, S, 128), bf16),
            pltpu.VMEM((M, DM), bf16),
            pltpu.VMEM((3, H // 2, DM, D), u32),
            pltpu.VMEM((3 * H, KP, D), bf16),
            pltpu.VMEM((H, KP, D), bf16),
            pltpu.VMEM((S, 2 * DM), bf16),
            pltpu.SemaphoreType.DMA((6,)),
            pltpu.SemaphoreType.DMA((2, 3)),
            pltpu.SemaphoreType.DMA((3, H // 2)),
            pltpu.SemaphoreType.DMA,
        ],
        compiler_params=pltpu.CompilerParams(vmem_limit_bytes=120 * 2**20),
    )(A_x.reshape(S, DM).T, A_c_kv.reshape(S, DC), A_w_q, A_w_uk, A_w_uv, jnp.swapaxes(A_w_o, 1, 2),
      B_x.reshape(S, DM).T, B_mem0.reshape(M, DM), B_Wq, B_Wk, B_Wv, jnp.swapaxes(B_Wo, 1, 2))
    return out.reshape(1, S, 2 * DM)
```

```python
import functools

import jax
import jax.numpy as jnp
import jax.experimental.pallas as pl
import jax.experimental.pallas.tpu as pltpu

f32, bf16, u32 = jnp.float32, jnp.bfloat16, jnp.uint32
NT = (((1,), (1,)), ((), ()))
LOG2E = 1.4426950408889634
BQ = 128
G = 2
FOLD_OUT = False
REV = False
LAG1, LAG2 = 1, 1


def _half(x, odd):
    y = (x >> (16 * odd).astype(u32)) << 16
    return pltpu.bitcast(y, f32).astype(bf16)


def _b(x):
    return pltpu.bitcast(x, bf16)


def _kernel(xa_hbm, c_hbm, wq_hbm, wuk_hbm, wuv_hbm, woa_hbm,
            xb_hbm, mem0_hbm, bq_hbm, bk_hbm, bv_hbm, wob_hbm,
            o_hbm,
            xt_s, xa_s, c_s, aw_s, woa_s, acc_s, ctx_s, xb_s, mem_s, bst_s, bw_s, wob_s, out_s,
            sem_in, sem_aw, sem_bw, sem_out):
    DM, S = xa_hbm.shape
    H, D = wq_hbm.shape[1], wq_hbm.shape[2]
    DC = c_hbm.shape[1]
    KP = 640
    PAD = KP - DM
    NK = KP // 128
    M = mem0_hbm.shape[0]
    cq = (D ** -0.5) * LOG2E

    aw32 = [w.bitcast(u32) for w in (wq_hbm, wuk_hbm, wuv_hbm)]
    bw32 = [w.bitcast(u32) for w in (bq_hbm, bk_hbm, bv_hbm)]

    def aw_copy(t, h, slot):
        k = aw32[t].shape[0]
        return pltpu.make_async_copy(aw32[t].at[:, h // 2, :], aw_s.at[slot, t, pl.ds(0, k), :],
                                     sem_aw.at[slot, t])

    def bw_copy(t, p):
        return pltpu.make_async_copy(bw32[t].at[:, p, :], bst_s.at[t, p], sem_bw.at[t, p])

    cp_xa = pltpu.make_async_copy(xa_hbm, xt_s.at[0, pl.ds(0, DM), :], sem_in.at[0])
    cp_c = pltpu.make_async_copy(c_hbm, c_s, sem_in.at[1])
    cp_woa = pltpu.make_async_copy(woa_hbm.bitcast(u32), woa_s.at[:, pl.ds(0, DM // 2), :], sem_in.at[2])
    cp_xb = pltpu.make_async_copy(xb_hbm, xt_s.at[1, pl.ds(PAD, DM), :], sem_in.at[3])
    cp_wob = pltpu.make_async_copy(wob_hbm.bitcast(u32), wob_s.at[:, pl.ds(PAD // 2, DM // 2), :], sem_in.at[4])
    cp_mem = pltpu.make_async_copy(mem0_hbm, mem_s, sem_in.at[5])

    cp_c.start()
    for t in (1, 2, 0):
        aw_copy(t, 0, 0).start()
    cp_xa.start()

    xt_s[0, DM:, :] = jnp.zeros((PAD, S), bf16)
    xt_s[1, :PAD, :] = jnp.zeros((PAD, S), bf16)
    woa_s[:, DM // 2:, :] = jnp.zeros((H, PAD // 2, D), u32)
    wob_s[:, :PAD // 2, :] = jnp.zeros((H, PAD // 2, D), u32)
    for sl in range(2):
        aw_s[sl, 0, DM:, :] = jnp.zeros((PAD, D), u32)
    cp_c.wait()
    cp_xa.wait()
    for p in range(H // 2):
        for t in range(3):
            bw_copy(t, p).start()
    cp_woa.start()
    cp_xb.start()
    cp_wob.start()
    cp_mem.start()
    for t in range(NK):
        for i in range(0, S, 256):
            xa_s[t, i:i + 256, :] = xt_s[0, t * 128:(t + 1) * 128, i:i + 256].T

    row = jax.lax.broadcasted_iota(jnp.int32, (BQ, BQ), 0)
    col = jax.lax.broadcasted_iota(jnp.int32, (BQ, BQ), 1)

    def head_body(h, carry):
        slot = h % 2
        odd = h % 2
        for t in range(3):
            aw_copy(t, h, slot).wait()

        @pl.when(h + 1 < H)
        def _():
            for t in range(3):
                aw_copy(t, h + 1, 1 - slot).start()

        @pl.when(odd == 0)
        def _():
            for t in range(3):
                bw_copy(t, h // 2).wait()

        cc = c_s[...]
        k = jnp.dot(cc, _half(aw_s[slot, 1, :DC, :], odd), preferred_element_type=f32).astype(bf16)
        v = jnp.dot(cc, _half(aw_s[slot, 2, :DC, :], odd), preferred_element_type=f32).astype(bf16)
        xx = jnp.concatenate([xa_s[t] for t in range(NK)], axis=1)
        q = jnp.dot(xx, _half(aw_s[slot, 0], odd), preferred_element_type=f32)
        q = (q * cq).astype(bf16)
        for t in range(3):
            bw_s[3 * h + t, pl.ds(0, PAD // 2), :] = jnp.zeros((PAD // 2, D), u32)
            bw_s[3 * h + t, pl.ds(PAD // 2, DM // 2), :] = pltpu.bitcast(_half(bst_s[t, h // 2], odd), u32)
        nb = S // BQ

        def qk_a(i):
            e = (i + 1) * BQ
            qi = q[i * BQ:e]
            sd = jax.lax.dot_general(qi, k[i * BQ:e], NT, preferred_element_type=f32)
            sd = jnp.where(col <= row, sd, -1e9)
            if i > 0:
                so = jax.lax.dot_general(qi, k[:i * BQ], NT, preferred_element_type=f32)
                return jnp.concatenate([so, sd], axis=1)
            return sd

        def sm_a(s):
            p = jnp.exp2(s - jnp.max(s, axis=1, keepdims=True))
            l = jnp.sum(p, axis=1, keepdims=True)
            return p.astype(bf16), pl.reciprocal(l, approx=False)

        def pv_a(i, p, r):
            e = (i + 1) * BQ
            o = (jnp.dot(p, v[:e], preferred_element_type=f32) * r).astype(bf16)
            ctx_s[h, i * BQ:e, :] = o

        order = list(range(nb)) if not REV else list(range(nb - 1, -1, -1))
        st = {}
        for t in range(nb + 2):
            if t < nb:
                st[('s', t)] = qk_a(order[t])
            if 0 <= t - LAG1 < nb:
                st[('p', t - LAG1)] = sm_a(st.pop(('s', t - LAG1)))
            if 0 <= t - LAG2 < nb:
                pv_a(order[t - LAG2], *st.pop(('p', t - LAG2)))
        return carry

    if FOLD_OUT:
        acc_s[...] = jnp.zeros(acc_s.shape, f32)
    with jax.named_scope('A_heads'):
        jax.lax.fori_loop(0, H, head_body, 0)
    if FOLD_OUT:
        out_s[:, :KP] = acc_s[...].astype(bf16)
    else:
        cp_woa.wait()

        def oa(i, carry):
            r = pl.ds(pl.multiple_of(i * 256, 256), 256)
            acc = None
            for h in range(H):
                t_ = jax.lax.dot_general(ctx_s[h, r, :], _b(woa_s[h]), NT, preferred_element_type=f32)
                acc = t_ if acc is None else acc + t_
            out_s[r, :KP] = acc.astype(bf16)
            return carry
        with jax.named_scope('A_out'):
            jax.lax.fori_loop(0, S // 256, oa, 0)

    cp_xb.wait()
    cp_wob.wait()
    cp_mem.wait()
    for t in range(NK):
        for i in range(0, S, 256):
            xb_s[t, i:i + 256, :] = xt_s[1, t * 128:(t + 1) * 128, i:i + 256].T

    L = 48
    r_ = jax.lax.broadcasted_iota(jnp.int32, (L, L), 0)
    c_ = jax.lax.broadcasted_iota(jnp.int32, (L, L), 1)
    maskA = ((r_ < 8) | (r_ >= c_)) & (c_ < 40)
    maskB = (((r_ >= 16) & (r_ < 24)) | ((c_ >= 16) & (c_ < 24)) | (r_ >= c_)) & (c_ >= 8)
    n = H // G

    def run(hh, mask, prevqkv, prevo):
        acc = [None]
        keep, keepo = {}, {}

        def proj(g):
            out = []
            for h in range(g * G, (g + 1) * G):
                q = (jnp.dot(hh, _b(bw_s[3 * h]), preferred_element_type=f32) * cq).astype(bf16)
                k = jnp.dot(hh, _b(bw_s[3 * h + 1]), preferred_element_type=f32).astype(bf16)
                v = jnp.dot(hh, _b(bw_s[3 * h + 2]), preferred_element_type=f32).astype(bf16)
                if prevqkv is None:
                    keep[h] = (q[32:48], k[32:48], v[32:48])
                else:
                    pq, pk, pv_ = prevqkv[h]
                    q = jnp.concatenate([pq, q], 0)
                    k = jnp.concatenate([pk, k], 0)
                    v = jnp.concatenate([pv_, v], 0)
                out.append((q, k, v))
            return out

        def qk(qkv):
            return [(jax.lax.dot_general(q, k, NT, preferred_element_type=f32), v) for q, k, v in qkv]

        def sm(sv):
            out = []
            for sc, v in sv:
                sc = jnp.where(mask, sc, -1e9)
                p = jnp.exp2(sc - jnp.max(sc, axis=1, keepdims=True))
                l = jnp.sum(p, axis=1, keepdims=True)
                out.append((p.astype(bf16), pl.reciprocal(l, approx=False), v))
            return out

        def pv(ps, g):
            out = []
            for j, (p, r, v) in enumerate(ps):
                h = g * G + j
                o = jnp.dot(p, v, preferred_element_type=f32) * r
                if prevo is None:
                    keepo[h] = o[32:40]
                    out.append(o[0:32].astype(bf16))
                else:
                    out.append(jnp.concatenate([prevo[h], o[8:48]], 0).astype(bf16))
            return out

        def wo(os, g):
            for j, o in enumerate(os):
                t_ = jax.lax.dot_general(o, _b(wob_s[g * G + j]), NT, preferred_element_type=f32)
                acc[0] = t_ if acc[0] is None else acc[0] + t_

        st = {}
        for t in range(n + 4):
            if t < n:
                st[('p', t)] = proj(t)
            if 0 <= t - 1 < n:
                st[('s', t - 1)] = qk(st.pop(('p', t - 1)))
            if 0 <= t - 2 < n:
                st[('m', t - 2)] = sm(st.pop(('s', t - 2)))
            if 0 <= t - 3 < n:
                st[('o', t - 3)] = pv(st.pop(('m', t - 3)), t - 3)
            if 0 <= t - 4 < n:
                wo(st.pop(('o', t - 4)), t - 4)
        return acc[0], keep, keepo

    def out_copy(j):
        r = pl.ds(pl.multiple_of(j * 64, 64), 64)
        return pltpu.make_async_copy(out_s.at[r, :], o_hbm.at[r, :], sem_out)

    def step(j, mem):
        r = pl.ds(pl.multiple_of(j * 64, 64), 64)
        X = jnp.concatenate([xb_s[t, r, :] for t in range(NK)], axis=1).astype(f32)
        hhA = jnp.concatenate([mem, X[0:40]], 0).astype(bf16)
        accA, keep, keepo = run(hhA, maskA, None, None)
        hhB = jnp.concatenate([accA[0:8], X[40:64]], 0).astype(bf16)
        accB, _, _ = run(hhB, maskB, keep, keepo)
        out = jnp.concatenate([accA[8:32], accB[0:16], accB[24:48]], 0)
        c0 = DM - PAD
        first = out[:, :128] + out_s[r, c0:c0 + 128].astype(f32)
        out_s[r, c0:c0 + 128] = first.astype(bf16)
        out_s[r, c0 + 128:] = out[:, 128:].astype(bf16)
        out_copy(j).start()
        return accB[16:24]

    mem0 = jnp.concatenate([jnp.zeros((M, PAD), f32), mem_s[...].astype(f32)], axis=1)
    with jax.named_scope('B_steps'):
        jax.lax.fori_loop(0, S // 64, step, mem0)
    pltpu.make_async_copy(out_s, o_hbm, sem_out).wait()


@functools.partial(jax.jit, static_argnames=("B_seg_len",))
def pallas_concat_heads__compressed_kv_cla__memory_aug_recurrent_mem_tr__prompt_kernel(
    A_x, A_c_kv, A_w_q, A_w_uk, A_w_uv, A_w_o,
    B_x, B_mem0, B_Wq, B_Wk, B_Wv, B_Wo, B_seg_len,
):
    Bn, S, DM = A_x.shape
    H, D = A_w_q.shape[1], A_w_q.shape[2]
    DC = A_c_kv.shape[2]
    M = B_mem0.shape[1]
    assert (Bn, DM, D, M, B_seg_len) == (1, 576, 128, 8, 32)
    KP = 640
    any_spec = pl.BlockSpec(memory_space=pl.ANY)
    out = pl.pallas_call(
        _kernel,
        out_shape=jax.ShapeDtypeStruct((S, 2 * DM), bf16),
        in_specs=[any_spec] * 12,
        out_specs=any_spec,
        scratch_shapes=[
            pltpu.VMEM((2, KP, S), bf16),
            pltpu.VMEM((KP // 128, S, 128), bf16),
            pltpu.VMEM((S, DC), bf16),
            pltpu.VMEM((2, 3, KP, D), u32),
            pltpu.VMEM((H, KP // 2, D), u32),
            pltpu.VMEM((S, KP), f32) if FOLD_OUT else pltpu.VMEM((8, 128), f32),
            pltpu.VMEM((8, 16, 128), bf16) if FOLD_OUT else pltpu.VMEM((H, S, D), bf16),
            pltpu.VMEM((KP // 128, S, 128), bf16),
            pltpu.VMEM((M, DM), bf16),
            pltpu.VMEM((3, H // 2, DM, D), u32),
            pltpu.VMEM((3 * H, KP // 2, D), u32),
            pltpu.VMEM((H, KP // 2, D), u32),
            pltpu.VMEM((S, 2 * DM), bf16),
            pltpu.SemaphoreType.DMA((6,)),
            pltpu.SemaphoreType.DMA((2, 3)),
            pltpu.SemaphoreType.DMA((3, H // 2)),
            pltpu.SemaphoreType.DMA,
        ],
        compiler_params=pltpu.CompilerParams(vmem_limit_bytes=120 * 2**20),
    )(A_x.reshape(S, DM).T, A_c_kv.reshape(S, DC), A_w_q, A_w_uk, A_w_uv, jnp.swapaxes(A_w_o, 1, 2),
      B_x.reshape(S, DM).T, B_mem0.reshape(M, DM), B_Wq, B_Wk, B_Wv, jnp.swapaxes(B_Wo, 1, 2))
    return out.reshape(1, S, 2 * DM)
```

```python
import functools

import jax
import jax.numpy as jnp
import jax.experimental.pallas as pl
import jax.experimental.pallas.tpu as pltpu

f32, bf16, u32 = jnp.float32, jnp.bfloat16, jnp.uint32
NT = (((1,), (1,)), ((), ()))
LOG2E = 1.4426950408889634
BQ = 128
G = 2
FOLD_OUT = False
TAIL = 5
PC, AHEAD = 128, 2
LAG1, LAG2 = 1, 1


def _half(x, odd):
    y = (x >> (16 * odd).astype(u32)) << 16
    return pltpu.bitcast(y, f32).astype(bf16)


def _b(x):
    return pltpu.bitcast(x, bf16)


def _kernel(xa_hbm, c_hbm, wq_hbm, wuk_hbm, wuv_hbm, woa_hbm,
            xb_hbm, mem0_hbm, bq_hbm, bk_hbm, bv_hbm, wob_hbm,
            o_hbm,
            xt_s, xa_s, c_s, aw_s, woa_s, acc_s, ctx_s, xb_s, mem_s, bst_s, bw_s, wob_s, out_s,
            sem_in, sem_aw, sem_bw, sem_out):
    DM, S = xa_hbm.shape
    H, D = wq_hbm.shape[1], wq_hbm.shape[2]
    DC = c_hbm.shape[1]
    KP = 640
    PAD = KP - DM
    NK = KP // 128
    M = mem0_hbm.shape[0]
    cq = (D ** -0.5) * LOG2E

    aw32 = [w.bitcast(u32) for w in (wq_hbm, wuk_hbm, wuv_hbm)]
    bw32 = [w.bitcast(u32) for w in (bq_hbm, bk_hbm, bv_hbm)]

    def aw_copy(t, h, slot):
        k = aw32[t].shape[0]
        return pltpu.make_async_copy(aw32[t].at[:, h // 2, :], aw_s.at[slot, t, pl.ds(0, k), :],
                                     sem_aw.at[slot, t])

    def bw_copy(t, p):
        return pltpu.make_async_copy(bw32[t].at[:, p, :], bst_s.at[t, p], sem_bw.at[t, p])

    cp_xa = pltpu.make_async_copy(xa_hbm, xt_s.at[0, pl.ds(0, DM), :], sem_in.at[0])
    cp_c = pltpu.make_async_copy(c_hbm, c_s, sem_in.at[1])
    cp_woa = pltpu.make_async_copy(woa_hbm.bitcast(u32), woa_s.at[:, pl.ds(0, DM // 2), :], sem_in.at[2])
    cp_xb = pltpu.make_async_copy(xb_hbm, xt_s.at[1, pl.ds(PAD, DM), :], sem_in.at[3])
    cp_wob = pltpu.make_async_copy(wob_hbm.bitcast(u32), wob_s.at[:, pl.ds(PAD // 2, DM // 2), :], sem_in.at[4])
    cp_mem = pltpu.make_async_copy(mem0_hbm, mem_s, sem_in.at[5])

    cp_c.start()
    for t in (1, 2, 0):
        aw_copy(t, 0, 0).start()
    cp_xa.start()

    xt_s[0, DM:, :] = jnp.zeros((PAD, S), bf16)
    xt_s[1, :PAD, :] = jnp.zeros((PAD, S), bf16)
    woa_s[:, DM // 2:, :] = jnp.zeros((H, PAD // 2, D), u32)
    wob_s[:, :PAD // 2, :] = jnp.zeros((H, PAD // 2, D), u32)
    for sl in range(2):
        aw_s[sl, 0, DM:, :] = jnp.zeros((PAD, D), u32)
    cp_c.wait()
    cp_xa.wait()
    for p in range(H // 2):
        for t in range(3):
            bw_copy(t, p).start()
    cp_woa.start()
    cp_xb.start()
    cp_wob.start()
    cp_mem.start()
    for t in range(NK):
        for i in range(0, S, 256):
            xa_s[t, i:i + 256, :] = xt_s[0, t * 128:(t + 1) * 128, i:i + 256].T

    row = jax.lax.broadcasted_iota(jnp.int32, (BQ, BQ), 0)
    col = jax.lax.broadcasted_iota(jnp.int32, (BQ, BQ), 1)

    def head_body(h, carry):
        slot = h % 2
        odd = h % 2
        for t in range(3):
            aw_copy(t, h, slot).wait()

        @pl.when(h + 1 < H)
        def _():
            for t in range(3):
                aw_copy(t, h + 1, 1 - slot).start()

        @pl.when(odd == 0)
        def _():
            for t in range(3):
                bw_copy(t, h // 2).wait()

        wk_ = _half(aw_s[slot, 1, :DC, :], odd)
        wv_ = _half(aw_s[slot, 2, :DC, :], odd)
        wq_ = _half(aw_s[slot, 0], odd)
        qs, ks, vs = [], [], []

        def proj_a(r0):
            cc = c_s[r0:r0 + PC, :]
            ks.append(jnp.dot(cc, wk_, preferred_element_type=f32).astype(bf16))
            xx = jnp.concatenate([xa_s[t, r0:r0 + PC, :] for t in range(NK)], axis=1)
            qs.append((jnp.dot(xx, wq_, preferred_element_type=f32) * cq).astype(bf16))
            vs.append(jnp.dot(cc, wv_, preferred_element_type=f32).astype(bf16))

        def rows(xs, a, b):
            out = []
            for j_, x in enumerate(xs):
                lo, hi = max(a, j_ * PC), min(b, (j_ + 1) * PC)
                if lo < hi:
                    out.append(x[lo - j_ * PC:hi - j_ * PC])
            return out[0] if len(out) == 1 else jnp.concatenate(out, axis=0)

        proj_a(0)
        for t in range(3):
            bw_s[3 * h + t, pl.ds(0, PAD // 2), :] = jnp.zeros((PAD // 2, D), u32)
            bw_s[3 * h + t, pl.ds(PAD // 2, DM // 2), :] = pltpu.bitcast(_half(bst_s[t, h // 2], odd), u32)
        nb = S // BQ

        def qk_a(i):
            e = (i + 1) * BQ
            qi = rows(qs, i * BQ, e)
            sd = jax.lax.dot_general(qi, rows(ks, i * BQ, e), NT, preferred_element_type=f32)
            sd = jnp.where(col <= row, sd, -1e9)
            if i > 0:
                so = jax.lax.dot_general(qi, rows(ks, 0, i * BQ), NT, preferred_element_type=f32)
                return jnp.concatenate([so, sd], axis=1)
            return sd

        def sm_a(s):
            p = jnp.exp2(s - jnp.max(s, axis=1, keepdims=True))
            l = jnp.sum(p, axis=1, keepdims=True)
            return p.astype(bf16), pl.reciprocal(l, approx=False)

        def pv_a(i, p, r):
            e = (i + 1) * BQ
            o = (jnp.dot(p, rows(vs, 0, e), preferred_element_type=f32) * r).astype(bf16)
            ctx_s[h, i * BQ:e, :] = o

        order = [0] + list(range(TAIL + 1, nb)) + list(range(TAIL, 0, -1))
        st = {}
        for t in range(nb + 2):
            while len(qs) * PC < min(S, (max(order[:t + 1]) + AHEAD) * BQ):
                proj_a(len(qs) * PC)
            if t < nb:
                st[('s', t)] = qk_a(order[t])
            if 0 <= t - LAG1 < nb:
                st[('p', t - LAG1)] = sm_a(st.pop(('s', t - LAG1)))
            if 0 <= t - LAG2 < nb:
                pv_a(order[t - LAG2], *st.pop(('p', t - LAG2)))
        return carry

    if FOLD_OUT:
        acc_s[...] = jnp.zeros(acc_s.shape, f32)
    with jax.named_scope('A_heads'):
        jax.lax.fori_loop(0, H, head_body, 0)
    if FOLD_OUT:
        out_s[:, :KP] = acc_s[...].astype(bf16)
    else:
        cp_woa.wait()

        def oa(i, carry):
            r = pl.ds(pl.multiple_of(i * 512, 512), 512)
            cc = jnp.concatenate([ctx_s[h, r, :] for h in range(H)], axis=1)
            for t in range(NK):
                nr = 64 if t < NK - 1 else (DM - 128 * t) // 2
                w = jnp.concatenate([_b(woa_s[h, 64 * t:64 * t + nr, :]) for h in range(H)], axis=1)
                ot = jax.lax.dot_general(w, cc, NT, preferred_element_type=f32).astype(bf16)
                if t == NK - 1:
                    ot = jnp.concatenate([ot, jnp.zeros((PAD, ot.shape[1]), bf16)], axis=0)
                out_s[r, 128 * t:128 * (t + 1)] = ot.T
            return carry
        with jax.named_scope('A_out'):
            jax.lax.fori_loop(0, S // 512, oa, 0)

    cp_xb.wait()
    cp_wob.wait()
    cp_mem.wait()
    for t in range(NK):
        for i in range(0, S, 256):
            xb_s[t, i:i + 256, :] = xt_s[1, t * 128:(t + 1) * 128, i:i + 256].T

    L = 48
    r_ = jax.lax.broadcasted_iota(jnp.int32, (L, L), 0)
    c_ = jax.lax.broadcasted_iota(jnp.int32, (L, L), 1)
    maskA = ((r_ < 8) | (r_ >= c_)) & (c_ < 40)
    maskB = (((r_ >= 16) & (r_ < 24)) | ((c_ >= 16) & (c_ < 24)) | (r_ >= c_)) & (c_ >= 8)
    n = H // G

    def run(hh, mask, prevqkv, prevo):
        acc = [None]
        keep, keepo = {}, {}

        def proj(g):
            out = []
            for h in range(g * G, (g + 1) * G):
                q = (jnp.dot(hh, _b(bw_s[3 * h]), preferred_element_type=f32) * cq).astype(bf16)
                k = jnp.dot(hh, _b(bw_s[3 * h + 1]), preferred_element_type=f32).astype(bf16)
                v = jnp.dot(hh, _b(bw_s[3 * h + 2]), preferred_element_type=f32).astype(bf16)
                if prevqkv is None:
                    keep[h] = (q[32:48], k[32:48], v[32:48])
                else:
                    pq, pk, pv_ = prevqkv[h]
                    q = jnp.concatenate([pq, q], 0)
                    k = jnp.concatenate([pk, k], 0)
                    v = jnp.concatenate([pv_, v], 0)
                out.append((q, k, v))
            return out

        def qk(qkv):
            return [(jax.lax.dot_general(q, k, NT, preferred_element_type=f32), v) for q, k, v in qkv]

        def sm(sv):
            out = []
            for sc, v in sv:
                sc = jnp.where(mask, sc, -1e9)
                p = jnp.exp2(sc - jnp.max(sc, axis=1, keepdims=True))
                l = jnp.sum(p, axis=1, keepdims=True)
                out.append((p.astype(bf16), pl.reciprocal(l, approx=False), v))
            return out

        def pv(ps, g):
            out = []
            for j, (p, r, v) in enumerate(ps):
                h = g * G + j
                o = jnp.dot(p, v, preferred_element_type=f32) * r
                if prevo is None:
                    keepo[h] = o[32:40]
                    out.append(o[0:32].astype(bf16))
                else:
                    out.append(jnp.concatenate([prevo[h], o[8:48]], 0).astype(bf16))
            return out

        def wo(os, g):
            for j, o in enumerate(os):
                t_ = jax.lax.dot_general(o, _b(wob_s[g * G + j]), NT, preferred_element_type=f32)
                acc[0] = t_ if acc[0] is None else acc[0] + t_

        st = {}
        for t in range(n + 4):
            if t < n:
                st[('p', t)] = proj(t)
            if 0 <= t - 1 < n:
                st[('s', t - 1)] = qk(st.pop(('p', t - 1)))
            if 0 <= t - 2 < n:
                st[('m', t - 2)] = sm(st.pop(('s', t - 2)))
            if 0 <= t - 3 < n:
                st[('o', t - 3)] = pv(st.pop(('m', t - 3)), t - 3)
            if 0 <= t - 4 < n:
                wo(st.pop(('o', t - 4)), t - 4)
        return acc[0], keep, keepo

    def out_copy(j):
        r = pl.ds(pl.multiple_of(j * 64, 64), 64)
        return pltpu.make_async_copy(out_s.at[r, :], o_hbm.at[r, :], sem_out)

    def step(j, mem):
        r = pl.ds(pl.multiple_of(j * 64, 64), 64)
        X = jnp.concatenate([xb_s[t, r, :] for t in range(NK)], axis=1).astype(f32)
        hhA = jnp.concatenate([mem, X[0:40]], 0).astype(bf16)
        accA, keep, keepo = run(hhA, maskA, None, None)
        hhB = jnp.concatenate([accA[0:8], X[40:64]], 0).astype(bf16)
        accB, _, _ = run(hhB, maskB, keep, keepo)
        out = jnp.concatenate([accA[8:32], accB[0:16], accB[24:48]], 0)
        c0 = DM - PAD
        first = out[:, :128] + out_s[r, c0:c0 + 128].astype(f32)
        out_s[r, c0:c0 + 128] = first.astype(bf16)
        out_s[r, c0 + 128:] = out[:, 128:].astype(bf16)
        out_copy(j).start()
        return accB[16:24]

    mem0 = jnp.concatenate([jnp.zeros((M, PAD), f32), mem_s[...].astype(f32)], axis=1)
    with jax.named_scope('B_steps'):
        jax.lax.fori_loop(0, S // 64, step, mem0)
    pltpu.make_async_copy(out_s, o_hbm, sem_out).wait()


@functools.partial(jax.jit, static_argnames=("B_seg_len",))
def pallas_concat_heads__compressed_kv_cla__memory_aug_recurrent_mem_tr__prompt_kernel(
    A_x, A_c_kv, A_w_q, A_w_uk, A_w_uv, A_w_o,
    B_x, B_mem0, B_Wq, B_Wk, B_Wv, B_Wo, B_seg_len,
):
    Bn, S, DM = A_x.shape
    H, D = A_w_q.shape[1], A_w_q.shape[2]
    DC = A_c_kv.shape[2]
    M = B_mem0.shape[1]
    assert (Bn, DM, D, M, B_seg_len) == (1, 576, 128, 8, 32)
    KP = 640
    any_spec = pl.BlockSpec(memory_space=pl.ANY)
    out = pl.pallas_call(
        _kernel,
        out_shape=jax.ShapeDtypeStruct((S, 2 * DM), bf16),
        in_specs=[any_spec] * 12,
        out_specs=any_spec,
        scratch_shapes=[
            pltpu.VMEM((2, KP, S), bf16),
            pltpu.VMEM((KP // 128, S, 128), bf16),
            pltpu.VMEM((S, DC), bf16),
            pltpu.VMEM((2, 3, KP, D), u32),
            pltpu.VMEM((H, KP // 2, D), u32),
            pltpu.VMEM((S, KP), f32) if FOLD_OUT else pltpu.VMEM((8, 128), f32),
            pltpu.VMEM((8, 16, 128), bf16) if FOLD_OUT else pltpu.VMEM((H, S, D), bf16),
            pltpu.VMEM((KP // 128, S, 128), bf16),
            pltpu.VMEM((M, DM), bf16),
            pltpu.VMEM((3, H // 2, DM, D), u32),
            pltpu.VMEM((3 * H, KP // 2, D), u32),
            pltpu.VMEM((H, KP // 2, D), u32),
            pltpu.VMEM((S, 2 * DM), bf16),
            pltpu.SemaphoreType.DMA((6,)),
            pltpu.SemaphoreType.DMA((2, 3)),
            pltpu.SemaphoreType.DMA((3, H // 2)),
            pltpu.SemaphoreType.DMA,
        ],
        compiler_params=pltpu.CompilerParams(vmem_limit_bytes=120 * 2**20),
    )(A_x.reshape(S, DM).T, A_c_kv.reshape(S, DC), A_w_q, A_w_uk, A_w_uv, jnp.swapaxes(A_w_o, 1, 2),
      B_x.reshape(S, DM).T, B_mem0.reshape(M, DM), B_Wq, B_Wk, B_Wv, jnp.swapaxes(B_Wo, 1, 2))
    return out.reshape(1, S, 2 * DM)
```

```python
import functools

import jax
import jax.numpy as jnp
import jax.experimental.pallas as pl
import jax.experimental.pallas.tpu as pltpu

f32, bf16, u32 = jnp.float32, jnp.bfloat16, jnp.uint32
NT = (((1,), (1,)), ((), ()))
LOG2E = 1.4426950408889634
BQ = 128
G = 2
FOLD_OUT = False
TAIL = 5
PC, AHEAD = 128, 2
LAG1, LAG2 = 1, 1


def _half(x, odd):
    y = (x >> (16 * odd).astype(u32)) << 16
    return pltpu.bitcast(y, f32).astype(bf16)


def _b(x):
    return pltpu.bitcast(x, bf16)


def _kernel(xa_hbm, c_hbm, wq_hbm, wuk_hbm, wuv_hbm, woa_hbm,
            xb_hbm, mem0_hbm, bq_hbm, bk_hbm, bv_hbm, wob_hbm,
            o_hbm,
            xt_s, xa_s, c_s, aw_s, woa_s, acc_s, ctx_s, xb_s, mem_s, bst_s, bw_s, wob_s, out_s,
            sem_in, sem_aw, sem_bw, sem_out):
    DM, S = xa_hbm.shape
    H, D = wq_hbm.shape[1], wq_hbm.shape[2]
    DC = c_hbm.shape[1]
    KP = 640
    PAD = KP - DM
    NK = KP // 128
    M = mem0_hbm.shape[0]
    cq = (D ** -0.5) * LOG2E

    aw32 = [w.bitcast(u32) for w in (wq_hbm, wuk_hbm, wuv_hbm)]
    bw32 = [w.bitcast(u32) for w in (bq_hbm, bk_hbm, bv_hbm)]

    def aw_copy(t, h, slot):
        k = aw32[t].shape[0]
        return pltpu.make_async_copy(aw32[t].at[:, h // 2, :], aw_s.at[slot, t, pl.ds(0, k), :],
                                     sem_aw.at[slot, t])

    def bw_copy(t, p):
        return pltpu.make_async_copy(bw32[t].at[:, p, :], bst_s.at[t, p], sem_bw.at[t, p])

    cp_xa = pltpu.make_async_copy(xa_hbm, xt_s.at[0, pl.ds(0, DM), :], sem_in.at[0])
    cp_c = pltpu.make_async_copy(c_hbm, c_s, sem_in.at[1])
    cp_woa = pltpu.make_async_copy(woa_hbm.bitcast(u32), woa_s.at[:, pl.ds(0, DM // 2), :], sem_in.at[2])
    cp_xb = pltpu.make_async_copy(xb_hbm, xt_s.at[1, pl.ds(PAD, DM), :], sem_in.at[3])
    cp_wob = pltpu.make_async_copy(wob_hbm.bitcast(u32), wob_s.at[:, pl.ds(PAD // 2, DM // 2), :], sem_in.at[4])
    cp_mem = pltpu.make_async_copy(mem0_hbm, mem_s, sem_in.at[5])

    cp_c.start()
    for t in (1, 2, 0):
        aw_copy(t, 0, 0).start()
    cp_xa.start()

    xt_s[0, DM:, :] = jnp.zeros((PAD, S), bf16)
    xt_s[1, :PAD, :] = jnp.zeros((PAD, S), bf16)
    woa_s[:, DM // 2:, :] = jnp.zeros((H, PAD // 2, D), u32)
    wob_s[:, :PAD // 2, :] = jnp.zeros((H, PAD // 2, D), u32)
    for sl in range(2):
        aw_s[sl, 0, DM:, :] = jnp.zeros((PAD, D), u32)
    cp_c.wait()
    cp_xa.wait()
    for t in range(3):
        bw_copy(t, 0).start()
    cp_mem.start()
    for t in range(NK):
        for i in range(0, S, 256):
            xa_s[t, i:i + 256, :] = xt_s[0, t * 128:(t + 1) * 128, i:i + 256].T

    row = jax.lax.broadcasted_iota(jnp.int32, (BQ, BQ), 0)
    col = jax.lax.broadcasted_iota(jnp.int32, (BQ, BQ), 1)

    def head_body(h, carry):
        slot = h % 2
        odd = h % 2
        for t in range(3):
            aw_copy(t, h, slot).wait()

        @pl.when(h + 1 < H)
        def _():
            for t in range(3):
                aw_copy(t, h + 1, 1 - slot).start()

        @pl.when(odd == 0)
        def _():
            for t in range(3):
                bw_copy(t, h // 2).wait()

            @pl.when(h + 2 < H)
            def _():
                for t in range(3):
                    bw_copy(t, h // 2 + 1).start()

        for hh_, cp in ((5, cp_woa), (9, cp_xb), (13, cp_wob)):
            @pl.when(h == hh_)
            def _():
                cp.start()

        wk_ = _half(aw_s[slot, 1, :DC, :], odd)
        wv_ = _half(aw_s[slot, 2, :DC, :], odd)
        wq_ = _half(aw_s[slot, 0], odd)
        qs, ks, vs = [], [], []

        def proj_a(r0):
            cc = c_s[r0:r0 + PC, :]
            ks.append(jnp.dot(cc, wk_, preferred_element_type=f32).astype(bf16))
            xx = jnp.concatenate([xa_s[t, r0:r0 + PC, :] for t in range(NK)], axis=1)
            qs.append((jnp.dot(xx, wq_, preferred_element_type=f32) * cq).astype(bf16))
            vs.append(jnp.dot(cc, wv_, preferred_element_type=f32).astype(bf16))

        def rows(xs, a, b):
            out = []
            for j_, x in enumerate(xs):
                lo, hi = max(a, j_ * PC), min(b, (j_ + 1) * PC)
                if lo < hi:
                    out.append(x[lo - j_ * PC:hi - j_ * PC])
            return out[0] if len(out) == 1 else jnp.concatenate(out, axis=0)

        proj_a(0)
        nb = S // BQ

        def qk_a(i):
            e = (i + 1) * BQ
            qi = rows(qs, i * BQ, e)
            sd = jax.lax.dot_general(qi, rows(ks, i * BQ, e), NT, preferred_element_type=f32)
            sd = jnp.where(col <= row, sd, -1e9)
            if i > 0:
                so = jax.lax.dot_general(qi, rows(ks, 0, i * BQ), NT, preferred_element_type=f32)
                return jnp.concatenate([so, sd], axis=1)
            return sd

        def sm_a(s):
            p = jnp.exp2(s - jnp.max(s, axis=1, keepdims=True))
            l = jnp.sum(p, axis=1, keepdims=True)
            return p.astype(bf16), pl.reciprocal(l, approx=False)

        def pv_a(i, p, r):
            e = (i + 1) * BQ
            o = (jnp.dot(p, rows(vs, 0, e), preferred_element_type=f32) * r).astype(bf16)
            ctx_s[h, i * BQ:e, :] = o

        order = [0] + list(range(TAIL + 1, nb)) + list(range(TAIL, 0, -1))
        st = {}
        for t in range(nb + 2):
            while len(qs) * PC < min(S, (max(order[:t + 1]) + AHEAD) * BQ):
                proj_a(len(qs) * PC)
            if t < nb:
                st[('s', t)] = qk_a(order[t])
            if 0 <= t - LAG1 < nb:
                st[('p', t - LAG1)] = sm_a(st.pop(('s', t - LAG1)))
            if 0 <= t - LAG2 < nb:
                pv_a(order[t - LAG2], *st.pop(('p', t - LAG2)))
        for t in range(3):
            bw_s[3 * h + t, pl.ds(0, PAD // 2), :] = jnp.zeros((PAD // 2, D), u32)
            bw_s[3 * h + t, pl.ds(PAD // 2, DM // 2), :] = pltpu.bitcast(_half(bst_s[t, h // 2], odd), u32)
        return carry

    if FOLD_OUT:
        acc_s[...] = jnp.zeros(acc_s.shape, f32)
    with jax.named_scope('A_heads'):
        jax.lax.fori_loop(0, H, head_body, 0)
    if FOLD_OUT:
        out_s[:, :KP] = acc_s[...].astype(bf16)
    else:
        cp_woa.wait()

        def oa(i, carry):
            r = pl.ds(pl.multiple_of(i * 512, 512), 512)
            cc = jnp.concatenate([ctx_s[h, r, :] for h in range(H)], axis=1)
            for t in range(NK):
                nr = 64 if t < NK - 1 else (DM - 128 * t) // 2
                w = jnp.concatenate([_b(woa_s[h, 64 * t:64 * t + nr, :]) for h in range(H)], axis=1)
                ot = jax.lax.dot_general(w, cc, NT, preferred_element_type=f32).astype(bf16)
                if t == NK - 1:
                    ot = jnp.concatenate([ot, jnp.zeros((PAD, ot.shape[1]), bf16)], axis=0)
                out_s[r, 128 * t:128 * (t + 1)] = ot.T
            return carry
        with jax.named_scope('A_out'):
            jax.lax.fori_loop(0, S // 512, oa, 0)

    cp_xb.wait()
    cp_wob.wait()
    cp_mem.wait()
    for t in range(NK):
        for i in range(0, S, 256):
            xb_s[t, i:i + 256, :] = xt_s[1, t * 128:(t + 1) * 128, i:i + 256].T

    L = 48
    r_ = jax.lax.broadcasted_iota(jnp.int32, (L, L), 0)
    c_ = jax.lax.broadcasted_iota(jnp.int32, (L, L), 1)
    maskA = ((r_ < 8) | (r_ >= c_)) & (c_ < 40)
    maskB = (((r_ >= 16) & (r_ < 24)) | ((c_ >= 16) & (c_ < 24)) | (r_ >= c_)) & (c_ >= 8)
    n = H // G

    def run(hh, mask, prevqkv, prevo):
        acc = [None]
        keep, keepo = {}, {}

        def proj(g):
            out = []
            for h in range(g * G, (g + 1) * G):
                q = (jnp.dot(hh, _b(bw_s[3 * h]), preferred_element_type=f32) * cq).astype(bf16)
                k = jnp.dot(hh, _b(bw_s[3 * h + 1]), preferred_element_type=f32).astype(bf16)
                v = jnp.dot(hh, _b(bw_s[3 * h + 2]), preferred_element_type=f32).astype(bf16)
                if prevqkv is None:
                    keep[h] = (q[32:48], k[32:48], v[32:48])
                else:
                    pq, pk, pv_ = prevqkv[h]
                    q = jnp.concatenate([pq, q], 0)
                    k = jnp.concatenate([pk, k], 0)
                    v = jnp.concatenate([pv_, v], 0)
                out.append((q, k, v))
            return out

        def qk(qkv):
            return [(jax.lax.dot_general(q, k, NT, preferred_element_type=f32), v) for q, k, v in qkv]

        def sm(sv):
            out = []
            for sc, v in sv:
                sc = jnp.where(mask, sc, -1e9)
                p = jnp.exp2(sc - jnp.max(sc, axis=1, keepdims=True))
                l = jnp.sum(p, axis=1, keepdims=True)
                out.append((p.astype(bf16), pl.reciprocal(l, approx=False), v))
            return out

        def pv(ps, g):
            out = []
            for j, (p, r, v) in enumerate(ps):
                h = g * G + j
                o = jnp.dot(p, v, preferred_element_type=f32) * r
                if prevo is None:
                    keepo[h] = o[32:40]
                    out.append(o[0:32].astype(bf16))
                else:
                    out.append(jnp.concatenate([prevo[h], o[8:48]], 0).astype(bf16))
            return out

        def wo(os, g):
            for j, o in enumerate(os):
                t_ = jax.lax.dot_general(o, _b(wob_s[g * G + j]), NT, preferred_element_type=f32)
                acc[0] = t_ if acc[0] is None else acc[0] + t_

        st = {}
        for t in range(n + 4):
            if t < n:
                st[('p', t)] = proj(t)
            if 0 <= t - 1 < n:
                st[('s', t - 1)] = qk(st.pop(('p', t - 1)))
            if 0 <= t - 2 < n:
                st[('m', t - 2)] = sm(st.pop(('s', t - 2)))
            if 0 <= t - 3 < n:
                st[('o', t - 3)] = pv(st.pop(('m', t - 3)), t - 3)
            if 0 <= t - 4 < n:
                wo(st.pop(('o', t - 4)), t - 4)
        return acc[0], keep, keepo

    def out_copy(j):
        r = pl.ds(pl.multiple_of(j * 64, 64), 64)
        return pltpu.make_async_copy(out_s.at[r, :], o_hbm.at[r, :], sem_out)

    def step(j, mem):
        r = pl.ds(pl.multiple_of(j * 64, 64), 64)
        X = jnp.concatenate([xb_s[t, r, :] for t in range(NK)], axis=1).astype(f32)
        hhA = jnp.concatenate([mem, X[0:40]], 0).astype(bf16)
        accA, keep, keepo = run(hhA, maskA, None, None)
        hhB = jnp.concatenate([accA[0:8], X[40:64]], 0).astype(bf16)
        accB, _, _ = run(hhB, maskB, keep, keepo)
        out = jnp.concatenate([accA[8:32], accB[0:16], accB[24:48]], 0)
        c0 = DM - PAD
        first = out[:, :128] + out_s[r, c0:c0 + 128].astype(f32)
        out_s[r, c0:c0 + 128] = first.astype(bf16)
        out_s[r, c0 + 128:] = out[:, 128:].astype(bf16)
        out_copy(j).start()
        return accB[16:24]

    mem0 = jnp.concatenate([jnp.zeros((M, PAD), f32), mem_s[...].astype(f32)], axis=1)
    with jax.named_scope('B_steps'):
        jax.lax.fori_loop(0, S // 64, step, mem0)
    pltpu.make_async_copy(out_s, o_hbm, sem_out).wait()


@functools.partial(jax.jit, static_argnames=("B_seg_len",))
def pallas_concat_heads__compressed_kv_cla__memory_aug_recurrent_mem_tr__prompt_kernel(
    A_x, A_c_kv, A_w_q, A_w_uk, A_w_uv, A_w_o,
    B_x, B_mem0, B_Wq, B_Wk, B_Wv, B_Wo, B_seg_len,
):
    Bn, S, DM = A_x.shape
    H, D = A_w_q.shape[1], A_w_q.shape[2]
    DC = A_c_kv.shape[2]
    M = B_mem0.shape[1]
    assert (Bn, DM, D, M, B_seg_len) == (1, 576, 128, 8, 32)
    KP = 640
    any_spec = pl.BlockSpec(memory_space=pl.ANY)
    out = pl.pallas_call(
        _kernel,
        out_shape=jax.ShapeDtypeStruct((S, 2 * DM), bf16),
        in_specs=[any_spec] * 12,
        out_specs=any_spec,
        scratch_shapes=[
            pltpu.VMEM((2, KP, S), bf16),
            pltpu.VMEM((KP // 128, S, 128), bf16),
            pltpu.VMEM((S, DC), bf16),
            pltpu.VMEM((2, 3, KP, D), u32),
            pltpu.VMEM((H, KP // 2, D), u32),
            pltpu.VMEM((S, KP), f32) if FOLD_OUT else pltpu.VMEM((8, 128), f32),
            pltpu.VMEM((8, 16, 128), bf16) if FOLD_OUT else pltpu.VMEM((H, S, D), bf16),
            pltpu.VMEM((KP // 128, S, 128), bf16),
            pltpu.VMEM((M, DM), bf16),
            pltpu.VMEM((3, H // 2, DM, D), u32),
            pltpu.VMEM((3 * H, KP // 2, D), u32),
            pltpu.VMEM((H, KP // 2, D), u32),
            pltpu.VMEM((S, 2 * DM), bf16),
            pltpu.SemaphoreType.DMA((6,)),
            pltpu.SemaphoreType.DMA((2, 3)),
            pltpu.SemaphoreType.DMA((3, H // 2)),
            pltpu.SemaphoreType.DMA,
        ],
        compiler_params=pltpu.CompilerParams(vmem_limit_bytes=120 * 2**20),
    )(A_x.reshape(S, DM).T, A_c_kv.reshape(S, DC), A_w_q, A_w_uk, A_w_uv, jnp.swapaxes(A_w_o, 1, 2),
      B_x.reshape(S, DM).T, B_mem0.reshape(M, DM), B_Wq, B_Wk, B_Wv, jnp.swapaxes(B_Wo, 1, 2))
    return out.reshape(1, S, 2 * DM)
```
